```python
import os as _os
_os.environ.setdefault("JAX_PLATFORMS", "cpu")
import jax
import jax.numpy as jnp

def _softmax(x, axis=-1):
    return jax.nn.softmax(x, axis=axis)
def _gelu(x):
    return jax.nn.gelu(x, approximate=True)
def _silu(x):
    return jax.nn.silu(x)
def _sigmoid(x):
    return jax.nn.sigmoid(x)
def _layernorm(x, axis=-1, eps=1e-5):
    m = jnp.mean(x, axis=axis, keepdims=True)
    v = jnp.var(x, axis=axis, keepdims=True)
    return (x - m) / jnp.sqrt(v + eps)
def _scatter_add(tgt, idx, src, axis=0):
    return tgt.at[idx].add(src)
def _segment_sum(src, seg, n):
    return jax.ops.segment_sum(src, seg, n)
class _Rng:
    def __init__(self, key):
        self._k = key
    def _next(self):
        self._k, sub = jax.random.split(self._k)
        return sub
    def normal(self, shape):
        return jax.random.normal(self._next(), shape, dtype=jnp.bfloat16)
    def randint(self, lo, hi, shape):
        return jax.random.randint(self._next(), shape, lo, hi, dtype=jnp.int32)
    def uniform(self, shape, lo=0.0, hi=1.0):
        return jax.random.uniform(self._next(), shape, jnp.bfloat16, lo, hi)
    def permutation(self, n):
        return jax.random.permutation(self._next(), n)


kernel_name = 'gated_mix__linear_kernel_hedgehog__mixer_s_mlp__prompt'

def setup_inputs():
    _rng = _Rng(jax.random.key(int.from_bytes(__import__("os").urandom(4), "little")))
    _w = (lambda a: (lambda t: t.astype(jnp.bfloat16) if jnp.issubdtype(t.dtype, jnp.floating) else t)(jnp.asarray(a)))
    def _A_setup():
        B, S, D, H = 1, 2048, 512, 32
        Dh = D // H
        return {
            "x": _w((lambda *s: _rng.normal(s) * 0.05)(B, S, D)),
            "wqkv": _w((lambda *s: _rng.normal(s) * 1.6)(D, 3 * D)),
            "w_phi": _w((lambda *s: _rng.normal(s) * 1.6)(H, Dh, Dh) * (Dh ** -0.5)),
            "wo": _w((lambda *s: _rng.normal(s) * 0.05)(D, D)),
        }
    _A_in = _A_setup()

    def _B_setup():
        B, S, D, F = 1, 2048, 512, 1376
        return {
            "x":  _w((lambda *s: _rng.normal(s) * 0.05)(B, S, D)),
            "w1": _w((lambda *s: _rng.normal(s) * 0.4)(D, D) * (D ** -0.5)),
            "w2": _w((lambda *s: _rng.normal(s) * 0.4)(D, D) * (D ** -0.5)),
            "w3": _w((lambda *s: _rng.normal(s) * 0.4)(D, F) * (D ** -0.5)),
            "w4": _w((lambda *s: _rng.normal(s) * 0.4)(F, D) * (F ** -0.5)),
        }
    _B_in = _B_setup()

    return {
        "A_x": _A_in["x"],
        "A_wqkv": _A_in["wqkv"],
        "A_w_phi": _A_in["w_phi"],
        "A_wo": _A_in["wo"],
        "B_x": _B_in["x"],
        "B_w1": _B_in["w1"],
        "B_w2": _B_in["w2"],
        "B_w3": _B_in["w3"],
        "B_w4": _B_in["w4"],
        "gate_w": _w((lambda *s: _rng.normal(s) * 0.05)(512) * 16.0),
    }

def reference(A_x, A_wqkv, A_w_phi, A_wo, B_x, B_w1, B_w2, B_w3, B_w4, gate_w):
    def _A_ref(x, wqkv, w_phi, wo):
        B, S, D = x.shape
        H = 32; Dh = D // H
        qkv = (lambda x, *d: x.transpose(*d))((x @ wqkv).reshape(B, S, 3, H, Dh), 2, 0, 3, 1, 4)
        q, k, v = qkv[0], qkv[1], qkv[2]
        pq = jnp.einsum("bhsd,hdf->bhsf", q, w_phi)
        pk = jnp.einsum("bhsd,hdf->bhsf", k, w_phi)
        phi_q = jnp.concatenate([_softmax(pq, axis=-1), _softmax(-pq, axis=-1)], axis=-1)
        phi_k = jnp.concatenate([_softmax(pk, axis=-1), _softmax(-pk, axis=-1)], axis=-1)
        kv = jnp.einsum("bhsf,bhsd->bhfd", phi_k, v)
        z  = jnp.einsum("bhsf->bhf", phi_k)
        num = jnp.einsum("bhqf,bhfd->bhqd", phi_q, kv)
        den = jnp.einsum("bhqf,bhf->bhq", phi_q, z)[..., None] + 1e-6
        o = num / den
        return (lambda x, *d: x.transpose(*d))(o, 0, 2, 1, 3).reshape(B, S, D) @ wo

    def _B_ref(x, w1, w2, w3, w4):
        B, S, D = x.shape
        h = _gelu(_layernorm(x, axis=-1) @ w1)
        c = D // 4
        g0 = jnp.pad(h[:, :, 0*c:1*c], ((0, 0), (1, 0), (0, 0)))[:, :S, :]
        g1 = jnp.pad(h[:, :, 1*c:2*c], ((0, 0), (0, 1), (0, 0)))[:, 1:, :]
        g2 = jnp.pad(h[:, :, 2*c:3*c], ((0, 0), (2, 0), (0, 0)))[:, :S, :]
        g3 = jnp.pad(h[:, :, 3*c:   ], ((0, 0), (0, 2), (0, 0)))[:, 2:, :]
        hs = jnp.concatenate([g0, g1, g2, g3], axis=-1) @ w2
        x1 = x + hs
        h2 = _gelu(_layernorm(x1, axis=-1) @ w3) @ w4
        return x1 + h2

    x = A_x
    g = _sigmoid((x * gate_w).sum(-1, keepdims=True))
    a = _A_ref(x, A_wqkv, A_w_phi, A_wo)
    b = _B_ref(x, B_w1, B_w2, B_w3, B_w4)
    return g * a + (1 - g) * b
```

```python
import functools
import jax
import jax.numpy as jnp
from jax import lax
import jax.experimental.pallas as pl
import jax.experimental.pallas.tpu as pltpu

S, D, H, DH, F = 2048, 512, 32, 16, 1376
FM = 1280
FT = F - FM
TM = 256
NB = S // TM
SH = (1, -1, 2, -2)
LOG2E = 1.4426950408889634
GC0 = 0.7978845608028654
GC1 = GC0 * 0.044715
NT = (((1,), (1,)), ((), ()))
f32 = jnp.float32
bf16 = jnp.bfloat16
u32 = jnp.uint32

_dot = functools.partial(jnp.dot, preferred_element_type=f32)
_dot_nt = functools.partial(lax.dot_general, dimension_numbers=NT, preferred_element_type=f32)


def _iota(shape, dim):
    return lax.broadcasted_iota(jnp.int32, shape, dim)


def _pack(x):
    return pltpu.bitcast(x.astype(bf16), u32)


def _unpack(x):
    return pltpu.bitcast(x, bf16)


def _ln(x):
    m = jnp.mean(x, axis=-1, keepdims=True)
    xc = x - m
    v = jnp.mean(xc * xc, axis=-1, keepdims=True)
    rs = jnp.exp2(-0.5 * jnp.log2(v + 1e-5))
    return x * rs - m * rs


def _gelu(u, scale):
    t = jnp.tanh(u * (GC0 + GC1 * (u * u)))
    hu = scale * u
    return hu + hu * t


def _swap4(a):
    return pltpu.roll(a, 4, 0)


def _zero_of(val, vrow):
    r = (vrow * 8) % val.shape[0]
    return pltpu.bitcast((pltpu.bitcast(val[r:r + 8, :128], u32) >> 16) >> 16, f32)


def _tie(t, zero):
    return jnp.concatenate([t[:8] + zero, t[8:]], axis=0)


def _dual_exp(p, zero=None):
    p3 = p.reshape(8, 8, p.shape[-1])
    mx = jnp.max(p3, axis=0)
    mn = jnp.min(p3, axis=0)
    mx = jnp.maximum(mx, _swap4(mx))
    mn = jnp.minimum(mn, _swap4(mn))
    if zero is not None:
        mx, mn = mx + zero, mn + zero
    ep = jnp.exp2(p3 - mx[None])
    en = jnp.exp2(mn[None] - p3)
    sp = jnp.sum(ep, axis=0)
    sn = jnp.sum(en, axis=0)
    return ep, en, sp + _swap4(sp), sn + _swap4(sn)


def _recip(x):
    r = pl.reciprocal(x, approx=True)
    return r * (2.0 - x * r)


def _quads(a):
    m, k = a.shape[0] // 2, a.shape[1] // 2
    return a[:m, :k], a[:m, k:], a[m:, :k], a[m:, k:]


def _join(c11, c12, c21, c22):
    return jnp.concatenate([jnp.concatenate([c11, c12], axis=1),
                            jnp.concatenate([c21, c22], axis=1)], axis=0)


LHS = (((0, 0, 1), (1, 1, 1)), ((1, 0, 1), (1, 1, 1)), ((0, 0, 1),), ((1, 1, 1),),
       ((0, 0, 1), (0, 1, 1)), ((1, 0, 1), (0, 0, -1)), ((0, 1, 1), (1, 1, -1)))
RHS = (((0, 0, 1), (1, 1, 1)), ((0, 0, 1),), ((0, 1, 1), (1, 1, -1)), ((1, 0, 1), (0, 0, -1)),
       ((1, 1, 1),), ((0, 0, 1), (0, 1, 1)), ((1, 0, 1), (1, 1, 1)))


def _comb(terms, q):
    t = q(*terms[0][:2])
    for a, b, sign in terms[1:]:
        t = t + q(a, b) if sign > 0 else t - q(a, b)
    return t


def _lhs7(*q):
    return [_comb(t, lambda a, b: q[2 * a + b]) for t in LHS]


def _rhs7(*q):
    return [_comb(t, lambda a, b: q[2 * a + b]) for t in RHS]


def _acc(d, acc):
    return d if acc is None else d + acc


def _strassen_steps(mul, order, acc, out):
    a11, a12, a21, a22 = acc if acc is not None else (None,) * 4
    r = {}
    for n, i in enumerate(order):
        if i == 2:
            r[2] = mul(1, a21)
        elif i == 3:
            r[3] = mul(2, a12)
        elif i == 4:
            r[4] = mul(3, r[2])
        elif i == 5:
            r[5] = mul(4, r[3])
        elif i == 1:
            r[1] = mul(0, r[3] - r[2])
        elif i == 6:
            r[6] = mul(5, r[1] if acc is None else r[1] + (a22 - a12 + a21))
        elif i == 7:
            r[7] = mul(6, _acc(r[1] + r[4] - r[5], a11))
        if n == 6:
            out((r[7], r[5], r[4], r[6]))
        yield


def _strassen(mul, order, acc):
    res = []
    for _ in _strassen_steps(mul, order, _quads(acc), res.append):
        pass
    return _join(*res[0])


ORD_N = (3, 2, 5, 4, 1, 6, 7)
ORD_T = (2, 3, 5, 4, 1, 6, 7)
ORD_2 = (2, 4, 3, 1, 6, 5, 7)
ORD_3 = (3, 2, 1, 6, 5, 4, 7)
GROUPS = (4, 5, 6, 7, 0, 1, 2, 3)

DMA = [["wk0"], ["wk1"], ["x0"], ["x1-2"], ["wv", "w1"], ["x3-4", "w3", "w2", "wo"], ["x5-7", "wq", "gw", "w4"]]
REGC = (
    "K1 s0 K2 s0 K1 K2 s0 K1 K2 s0 K1 K1 s0 K2 s0 K1 K2 K2 K1 s0 K2 s0"
)
REGD = (
    "u0:8 u0:6 u0:8 u0:3 V0 s1 s1 V1 V1:4 V0 s1 V1 V0:2 V0 V1 s1 s1 s1 s1 V0 V1 V0 V1 V1:1 V0 U1 b0 U1 b0 "
    "s1 b0 b0 U1 U1 U1 b0 U1 s2 U1 b0 b0 w2 b1 w2 b1 s2 b0 w2 b1 s2 s2 b1 b1 w2 b1 w2 w2 b1 w2 b1 U2 b2 "
    "U2 U2 U2 U2 U2 b2 U2 b2 b2"
)
REGE = (
    "K3:5 V3:8 b2 K3:8 V3:8 b2 b2 K3:8 V3:7 K3:8 V3:8 b2 K3 V3 K3 V3 K3:1 V3 U3:1 U3 U3 U3 U3 U3:1 b3 b3 "
    "b3 U3 b3 K4:8 V4:7 b3 s3 V4:9 K4:8 b3 b3 V4:8 K4:8 K4:7 V4:8 K4 V4 K4:1 V4:2 b3 K4 V4 U4 U4 U4 U4 b4 "
    "U4 U4 U4:1 b4 b4 b4"
)
REGF = (
    "K5:8 V5:8 b4 V5:8 K5:8 b4 K5:8 V5:7 b4 K5:9 V5:8 b4 K5 V5 V5 K5 V5 K5:1 U5 b5 U5:1 U5:1 b5 U5 U5:1 "
    "b5 b5 U5 U5 b5 K6:7 V6:9 K6:5 b5 V6:8 K6:7 K6:6 V6:8 V6:7 b5 K6 V6 b5 K6 V6 K6:1 V6 U6 U6 U6 U6 U6 "
    "b6 U6 U6 b6 s6 b6 b6 K7:8 b6 V7:8 s6 K7:8 K7:8 V7:6 V7:8 b6 b6 K7:8 V7:6 V7 K7 K7 V7 K7:3 U7 b6 V7 "
    "U7:2 b7 U7 b7 U7 b7 U7 U7 U7 b7 b7 s7 b7 b7 b7 F F F F:1"
)
SEQ2 = (
    "A0 G0 A0 P0 G0 A0x4 G0 A0 P0 B0x5 G0 B0x7 N0 B0x2 N0x3 B0x6 N0 B0x2 A1 N0 B0x3 G1x2 N0 A1 N0 G1 A1 "
    "G1 A1x2 B0x9 A1 B0x2 A1 C0x2 P1 C0x4 P1 C0 B1x21 N1x3 B1 N1x5 B1x7 G2 B1x4 A2 B1 G2 B1x2 A2 G2x2 A2 "
    "C1 A2x4 C1x2 P2x2 C1 B2 C1x2 B2x3 C1 B2x4 N2 B2x8 N2 B2x4 N2 B2 A3 B2x7 N2 G3 B2x3 A3 B2 N2 A3 N2 "
    "B2x2 N2x2 B2x2 A3x4 C2x3 P3x2 G3x3 C2x2 B3x8 C2x2 N3 B3x7 N3 B3x5 N3 B3x2 N3x4 B3x5 N3 B3x9 C3x7"
)


PLAN = " ".join(["| G0 | G1 | k0 k0 k0 k0 k0 k0 k0 l0 |", REGC, "| T +w1", REGD, "| +w3 +w2 +wo", REGE,
                 "| +w4", REGF])
N2 = 4


def build(checks=False):
    def kernel(x_hbm, wqkv_hbm, wphi_hbm, wo_hbm, w1_hbm, w2_hbm, w3t_hbm, w4_hbm, gw_hbm,
               o_hbm,
               x_ref, wq_ref, wk_ref, wv_ref, wphi_ref, wo_ref, w1_ref, w2_ref, w3t_ref, w4_ref, gw_ref,
               o_ref, mt_ref, wqt_ref, lk_ref, lv_ref, h_ref, kv_ref, z_ref, kvm_ref, st_ref,
               r1_ref, r2_ref, r3_ref, r4_ref, ro_ref, rd_ref, lh0_ref, lh1_ref, zero_ref,
               sem):
        cp = pltpu.make_async_copy

        def mkdma(name, s):
            if name[0] == "x":
                lo, hi = int(name[1]), int(name[-1]) + 1
                rows = pl.ds(lo * TM, (hi - lo) * TM)
                return [cp(x_hbm.at[rows, :], x_ref.at[rows, :], s)]
            if name in ("wk0", "wk1"):
                g = int(name[-1])
                return [cp(wqkv_hbm.at[:, pl.ds(D + gg * 128, 128)], wk_ref.at[:, pl.ds(gg * 128, 128)], s)
                        for gg in (g, g + 2)]
            src, dst = {
                "wq": (wqkv_hbm.at[:, pl.ds(0, D)], wq_ref), "wv": (wqkv_hbm.at[:, pl.ds(2 * D, D)], wv_ref),
                "w1": (w1_hbm, w1_ref), "w2": (w2_hbm, w2_ref), "w3": (w3t_hbm, w3t_ref),
                "w4": (w4_hbm, w4_ref), "wo": (wo_hbm, wo_ref), "gw": (gw_hbm, gw_ref),
            }[name]
            return [cp(src, dst, s)]

        def slot(n, rows, r=0, size=None):
            return pl.ds((n // 2 * rows + r) // 2, (size or rows) // 2), pl.ds(n % 2 * 128, 128)

        def prep1(w_ref, dst, nr, nt=False, scale=None, lo=0):
            def chunk(r, c, zero):
                q = lambda i, j: w_ref[pl.ds(i * nr + r, 16), pl.ds(j * 256 + c, 128)].astype(f32)
                qs = [q(0, 0), q(1, 0), q(0, 1), q(1, 1)] if nt else [q(0, 0), q(0, 1), q(1, 0), q(1, 1)]
                if scale is not None:
                    qs = [t * scale for t in qs]
                qs[0], qs[3] = _tie(qs[0], zero), _tie(qs[3], zero)
                for i, t in enumerate(_rhs7(*qs)):
                    dst[pl.ds((i * (nr - lo) + r - lo) // 2, 8), pl.ds(c, 128)] = _pack(t)

            return [functools.partial(chunk, r, c) for r in range(lo, nr, 16) for c in (0, 128)]

        def prep2(w_ref, dst, k, ki, scale=None, flip=False):
            def chunk(i, r, zero):
                def q(a, b):
                    col = lambda y: 3 - (2 * y + b) if flip else 2 * y + b
                    t = _comb(RHS[i], lambda x, y: w_ref[pl.ds(x * k + a * ki + r, 16),
                                                         pl.ds(col(y) * 128, 128)].astype(f32))
                    return t if scale is None else t * scale
                qs = [q(0, 0), q(0, 1), q(1, 0), q(1, 1)]
                qs[0], qs[3] = _tie(qs[0], zero), _tie(qs[3], zero)
                for j, t in enumerate(_rhs7(*qs)):
                    dst[slot(i * 7 + j, ki, r, 16)] = _pack(t)

            return [functools.partial(chunk, i, r) for i in range(7) for r in range(0, ki, 16)]

        pending = []
        last = [None]
        npin = [0]

        def tick(val):
            n = npin[0]
            last[0] = val
            for k in range(n):
                if pending:
                    pending.pop(0)(_zero_of(val, k * (val.shape[0] // 8) // n))
            return val

        def key_pass():
            c_wphi = cp(wphi_hbm, wphi_ref, sem.at[0])
            stages = [sum([mkdma(nm, sem.at[2 + n]) for nm in st], []) for n, st in enumerate(DMA)]
            for c in [c_wphi] + sum(stages[:-1], []):
                c.start()

            zero_ref[0] = 0
            kv_ref[...] = jnp.zeros_like(kv_ref)
            h_ref[:, pl.ds(0, 16), :] = jnp.zeros((4, 16, 128), f32)
            h_ref[:, pl.ds(S, 16), :] = jnp.zeros((4, 16, 128), f32)

            c_wphi.wait()
            for c in stages[-1]:
                c.start()
            wp = wphi_ref[...].reshape(DH * DH, H)
            rep = jnp.where(_iota((H, D), 1) // DH == _iota((H, D), 0), 1.0, 0.0).astype(bf16)
            b = _dot(wp, rep).reshape(DH, DH, D)
            b = jnp.where(_iota((DH, DH, D), 0) == _iota((DH, DH, D), 2) % DH, b, 0.0)
            cmat = jnp.sum(b, axis=0).astype(bf16)
            r = _iota((128, DH), 0)
            e = jnp.where((r % 64) // 4 == _iota((128, DH), 1), 1.0, 0.0).astype(bf16)
            t = _dot(e, cmat)
            r = _iota((128, D), 0)
            c = _iota((128, D), 1)
            mt_ref[...] = _pack(jnp.where((r // 64) * 4 + r % 4 == (c // DH) % 8, t, 0.0))

            def fold(w_ref, g):
                cols = slice(g * 128, (g + 1) * 128)
                return _dot_nt(_unpack(mt_ref[:, cols]), w_ref[:, cols]) * LOG2E

            def fold_k(g):
                top, bot = fold(wk_ref, g), fold(wk_ref, g + 2)
                for i, t in enumerate(_lhs7(top[:, :256], top[:, 256:], bot[:, :256], bot[:, 256:])):
                    lk_ref[pl.ds(i * 128 + g * 64, 64), :] = _pack(t)

            def tasks_of(i):
                r0 = i * TM
                v = {}

                def xr():
                    if "xr" not in v:
                        xb = x_ref[pl.ds(r0, TM), :]
                        q11, q21, q12, q22 = _quads(xb.astype(f32))
                        r7 = [t.astype(bf16) for t in _rhs7(q11, q12, q21, q22)]
                        r7[1], r7[4] = xb[:128, :256], xb[128:, 256:]
                        v["xr"] = r7
                    return v["xr"]

                def tmm(l_ref, name, split):
                    def mul(i, c):
                        if split and i == ORD_T[-1] - 1:
                            return jnp.concatenate(
                                [_dot_nt(_unpack(l_ref[pl.ds(i * 128 + h * 64, 64), :]), xr()[i])
                                 + c[h * 128:(h + 1) * 128] for h in range(2)], axis=0)
                        return tick(_acc(_dot_nt(_unpack(l_ref[pl.ds(i * 128, 128), :]), xr()[i]), c))
                    return _strassen_steps(mul, ORD_T, None, lambda c: v.update({name: _join(*c)}))

                def ln():
                    return _ln(x_ref[pl.ds(r0, TM), :].astype(f32))

                def l_steps():
                    v["xn"] = ln().astype(bf16)
                    yield

                def store_h(c, uu):
                    h_ref[c, pl.ds(r0 + 8 + SH[c], TM), :] = _gelu(uu, 0.5)

                def ustd_steps():
                    for c in range(4):
                        store_h(c, tick(_dot(v["xn"], w1_ref[:, pl.ds(c * 128, 128)])))
                        yield

                def u_steps():
                    l = [t.astype(bf16) for t in _lhs7(*_quads(ln()))]
                    mul = lambda i, c: tick(_acc(_dot(l[i], _unpack(r1_ref[pl.ds(i * 128, 128), :])), c))

                    def done(q):
                        uu = _join(*q)
                        for c in range(4):
                            store_h(c, uu[:, c * 128:(c + 1) * 128])

                    yield from _strassen_steps(mul, ORD_N, None, done)

                def phi(g, anchor):
                    if ("ph", g) not in v:
                        zero = None
                        if anchor is not None:
                            zero = jnp.concatenate([_zero_of(anchor, 0), _zero_of(anchor, 16)], axis=1)
                        ep, en, sp, sn = _dual_exp(v["pk"][g * 64:(g + 1) * 64], zero)
                        ph = jnp.concatenate([ep * _recip(sp)[None], en * _recip(sn)[None]], axis=0)
                        v["ph", g] = ph.reshape(128, TM).astype(bf16)
                    return v["ph", g]

                def s_steps():
                    for g in GROUPS:
                        phi(g, last[0])
                        yield

                def kv_steps():
                    for g in GROUPS:
                        vg = jnp.concatenate([v["vt"][g * 64:(g + 1) * 64], jnp.ones((16, TM), f32)], axis=0)
                        kv_ref[g] += _dot_nt(vg.astype(bf16), phi(g, None))
                        yield

                return dict(K=tmm(lk_ref, "pk", False), k=tmm(lk_ref, "pk", True), V=tmm(lv_ref, "vt", False),
                            w=tmm(lv_ref, "vt", True), U=u_steps(), u=ustd_steps(), b=kv_steps(), s=s_steps(),
                            l=l_steps())

            tasks = [tasks_of(i) for i in range(NB)]
            preps = {
                "+w1": lambda: prep1(w1_ref, r1_ref, 256),
                "+w2": lambda: prep2(w2_ref, r2_ref, 256, 128, flip=True),
                "+w3": lambda: prep1(w3t_ref, r3_ref, FM // 2, nt=True),
                "+w4": lambda: (prep1(w4_ref, rd_ref, FM // 2, scale=0.5, lo=512)
                                + prep2(w4_ref, r4_ref, FM // 2, 256, scale=0.5)),
                "+wo": lambda: prep2(wo_ref, ro_ref, 256, 128),
            }
            count = {}
            for tok in PLAN.split():
                tok, _, n = tok.partition(":")
                npin[0] = int(n or 0)
                seen = count.get(tok, 0)
                count[tok] = seen + 1
                if tok == "+w3" or (tok[0] == "U" and "+w3" not in count):
                    assert not pending, "w1 operands not ready"
                if tok == "|":
                    for c in stages[seen]:
                        c.wait()
                    last[0] = None
                elif tok[0] == "+":
                    pending.extend(preps[tok]())
                elif tok[0] == "G":
                    fold_k(int(tok[1]))
                elif tok == "F":
                    wqt_ref[pl.ds(seen * 64, 64), :] = _pack(tick(fold(wq_ref, seen)))
                elif tok == "T":
                    for i, t in enumerate(_lhs7(*_quads(wv_ref[...].astype(f32).T))):
                        lv_ref[pl.ds(i * 128, 128), :] = _pack(t)
                else:
                    next(tasks[int(tok[1])][tok[0]])
            npin[0] = 0
            assert count["|"] == len(DMA) and not pending and count["F"] == 4
            for i in range(NB):
                c = lambda ch: count.get("%s%d" % (ch, i), 0)
                assert c("K") + c("k") == 7 and c("V") + c("w") == 7 and c("b") == 8
                assert c("U") == 7 or c("u") == 4
            own = _iota((64, 128), 0) // DH == _iota((64, 128), 1) % 4
            for g in range(8):
                kvm_ref[slot(g, 64)] = _pack(jnp.where(own, kv_ref[g, pl.ds(0, 64), :], 0.0))
                z_ref[g] = jnp.concatenate([kv_ref[g, pl.ds(64, 8), :]] * 16, axis=0).T

        def out_tasks(i, is_last, dz, lh_ref):
            r0 = pl.multiple_of(i * TM, TM)
            v = {}

            def logit(q, anchor):
                if ("lg", q) not in v:
                    st_ref[0] = jnp.zeros((8, 128), f32)
                    gw = gw_ref[...].astype(f32).reshape(1, D) * 0.5
                    t = x_ref[pl.ds(r0 + q * 64, 64), :].astype(f32) * gw
                    t = (t[:, :128] + t[:, 128:256]) + (t[:, 256:384] + t[:, 384:])
                    if anchor is not None:
                        nv = anchor.shape[0] // 8
                        t = t + jnp.concatenate([_zero_of(anchor, k // 2 * nv // 4) for k in range(8)], axis=0)
                    v["lg", q] = jnp.sum(t, axis=-1, keepdims=True)
                    st_ref[1] = jnp.zeros((8, 128), f32)
                return v["lg", q]

            def g_steps():
                for q in range(4):
                    logit(q, last[0])
                    yield

            def omg():
                if "omg" not in v:
                    v["omg"] = 0.5 - 0.5 * jnp.tanh(jnp.concatenate([logit(q, None) for q in range(4)], axis=0))
                return v["omg"]

            def a_steps():
                xb = x_ref[pl.ds(r0, TM), :].astype(f32)
                blk = lambda a, c: h_ref[c, pl.ds(r0 + 8 + a * 64, 64), :]

                def mul(i, c):
                    def inner(j, cc):
                        t = _comb(LHS[j], lambda a2, b2: _comb(LHS[i], lambda a1, b1: blk(a1 * 2 + a2, b1 * 2 + b2)))
                        return _dot(t.astype(bf16), _unpack(r2_ref[slot(i * 7 + j, 128)])) + cc
                    return tick(_strassen(inner, ORD_N, c))

                flip = lambda t: jnp.concatenate([t[:, (3 - c) * 128:(4 - c) * 128] for c in range(4)], axis=1)
                yield from _strassen_steps(mul, ORD_2, _quads(flip(xb)), lambda c: v.update(x1=flip(_join(*c))))

            def p_steps():
                for c in range(2):
                    v["pq", c] = tick(_dot_nt(_unpack(wqt_ref[...]), x_ref[pl.ds(r0 + c * 128, 128), :]))
                    yield

            def b_steps():
                q = _quads(_ln(v["x1"]))
                l = [t.astype(bf16) for t in _lhs7(*q) + [q[1], q[2]]]
                for j in range(5):
                    mul = lambda i, c: tick(_acc(
                        _dot_nt(l[i], _unpack(r3_ref[pl.ds(i * (FM // 4) + j * 64, 64), :])), c))

                    def done(c):
                        om = omg()
                        hq = (_gelu(c[0], om[:128]), _gelu(c[1], om[:128]),
                              _gelu(c[2], om[128:]), _gelu(c[3], om[128:]))
                        for i, t in enumerate(_lhs7(*hq)):
                            lh_ref[pl.ds(i * 64, 64), pl.ds(j * 128, 128)] = _pack(t)

                    yield from _strassen_steps(mul, ORD_3, None, done)
                w = lambda h: w3t_ref[pl.ds(FM, FT), pl.ds(h * 256, 256)]
                ut = jnp.concatenate([_dot_nt(w(1), l[7]) + _dot_nt(w(0), l[2]),
                                      _dot_nt(w(1), l[3]) + _dot_nt(w(0), l[8])], axis=1)
                v["ut"] = jnp.concatenate([ut, jnp.zeros((128 - FT, TM), f32)], axis=0).T[:, :FT]
                yield

            def n_steps():
                ots = {}
                gate = 1.0 - jnp.broadcast_to(omg(), (TM, 128)).T[0:8]
                for c in range(2):
                    for g in range(8):
                        ep, en, sp, sn = _dual_exp(v["pq", c][g * 64:(g + 1) * 64])
                        zb = z_ref[g].reshape(16, 8, 128)
                        tp = jnp.sum(ep * zb[0:8], axis=0)
                        tn = jnp.sum(en * zb[8:16], axis=0)
                        den = tp * sn + tn * sp
                        rd = _recip(den + _swap4(den) + 1e-6 * (sp * sn)) * gate[:, c * 128:(c + 1) * 128]
                        ph = jnp.concatenate([ep * (sn * rd)[None], en * (sp * rd)[None]], axis=0)
                        ots[g, c] = _dot(_unpack(kvm_ref[slot(g, 64)]), ph.reshape(128, 128).astype(bf16))
                        if (g, c) == (7, 1):
                            o = jnp.concatenate(
                                [jnp.concatenate([ots[k, 0], ots[k, 1]], axis=1) for k in range(8)], axis=0).T
                            v["lo"] = _lhs7(*_quads(o))
                        if g % 2 == 1:
                            yield

            def c_steps():
                ht = _gelu(v["ut"], omg()) * 0.5
                ox11, ox12, ox21, ox22 = _quads(omg() * v["x1"])

                def mul(i, c):
                    hq = lambda a, b: _unpack(lh_ref[pl.ds(dz + i * 64 + a * 32, 32), pl.ds(b * 256, 256)])

                    def inner(j, cc):
                        st_ref[0] = jnp.zeros((8, 128), f32)
                        n = i * 7 + j
                        do = _dot(_lhs7(*_quads(v["lo"][i]))[j].astype(bf16), _unpack(ro_ref[slot(n, 128)]))
                        lh = (hq(*LHS[j][0][:2]) if len(LHS[j]) == 1
                              else _comb(LHS[j], lambda a, b: hq(a, b).astype(f32)).astype(bf16))
                        return do + (_dot(lh, _unpack(r4_ref[slot(n, 256)])) + cc)

                    direct = _acc(_dot(_unpack(lh_ref[pl.ds(dz + i * 64, 64), pl.ds(512, 128)]),
                                       _unpack(rd_ref[pl.ds(i * 64, 64), :])), c)
                    return tick(_strassen(inner, ORD_N, direct))

                def tail(r, c, a):
                    return _dot(ht[r * 128:(r + 1) * 128].astype(bf16),
                                w4_ref[pl.ds(FM, FT), pl.ds(c * 256, 256)]) + a

                def emit(row, col, y):
                    at = (pl.ds(r0 + row, y.shape[0]), pl.ds(col, y.shape[1]))
                    o_ref[at] = y.astype(o_ref.dtype)
                    cp(o_ref.at[at], o_hbm.at[at], sem.at[1]).start()

                m3 = mul(2, None)
                yield
                m2 = mul(1, None)
                yield
                c12 = mul(4, m3)
                yield
                c21 = mul(3, m2)
                yield
                u = mul(0, m3 - m2)
                yield
                y21 = tail(1, 0, c21 + ox21)
                y22 = mul(5, tail(1, 1, u + ox22))
                emit(128, 0, jnp.concatenate([y21, y22], axis=1))
                yield
                y12 = tail(0, 1, c12 + ox12)
                t11 = tail(0, 0, u + c21 - c12 + ox11)
                if is_last:
                    emit(0, 256, y12)
                    y11 = mul(6, t11)
                    emit(0, 128, y11[:64, 128:])
                    emit(64, 0, y11[64:])
                    emit(0, 0, y11[:64, :128])
                else:
                    emit(0, 0, jnp.concatenate([mul(6, t11), y12], axis=1))
                yield

            return dict(P=p_steps(), A=a_steps(), B=b_steps(), N=n_steps(), C=c_steps(), G=g_steps())

        def outer(k, carry):
            pl.when(k == 0)(key_pass)
            dz = pl.multiple_of(zero_ref[0], 32)
            ts = [out_tasks(k * N2 + j, j == N2 - 1, dz, (lh0_ref, lh1_ref)[j % 2]) for j in range(N2)]
            last[0] = None
            done = {}
            need = dict(P=2, A=7, B=36, N=8, C=7)
            for tok in SEQ2.split():
                t, j, n = tok[0], int(tok[1]), int(tok[3:] or 1)
                if t == "B" and j >= 2:
                    assert done.get("C%d" % (j - 2), 0) == need["C"]
                if t == "C":
                    assert done.get("B%d" % j, 0) == need["B"] and done.get("N%d" % j, 0) == need["N"]
                for _ in range(n):
                    next(ts[j][t])
                done[tok[:2]] = done.get(tok[:2], 0) + n
            assert all(done.get("%s%d" % (t, j), 0) == c for t, c in need.items() for j in range(N2))
            return carry

        lax.fori_loop(0, NB // N2, outer, 0)
        cp(o_ref, o_hbm, sem.at[1]).wait()

    @jax.jit
    def run(A_x, A_wqkv, A_w_phi, A_wo, B_x, B_w1, B_w2, B_w3, B_w4, gate_w):
        hbm = pl.BlockSpec(memory_space=pl.ANY)
        out = pl.pallas_call(
            kernel,
            out_shape=jax.ShapeDtypeStruct((S, D), A_x.dtype),
            in_specs=[hbm] * 9,
            out_specs=hbm,
            scratch_shapes=[
                pltpu.VMEM((S, D), bf16),
                pltpu.VMEM((D, D), bf16),
                pltpu.VMEM((D, D), bf16),
                pltpu.VMEM((D, D), bf16),
                pltpu.VMEM((DH, DH, H), bf16),
                pltpu.VMEM((D, D), bf16),
                pltpu.VMEM((D, D), bf16),
                pltpu.VMEM((D, D), bf16),
                pltpu.VMEM((F, D), bf16),
                pltpu.VMEM((F, D), bf16),
                pltpu.VMEM((D,), bf16),
                pltpu.VMEM((S, D), bf16),
                pltpu.VMEM((64, D), u32),
                pltpu.VMEM((D // 2, D), u32),
                pltpu.VMEM((7 * 128, 256), u32),
                pltpu.VMEM((7 * 128, 256), u32),
                pltpu.VMEM((4, S + 16, 128), f32),
                pltpu.VMEM((8, 80, 128), f32),
                pltpu.VMEM((8, 128, 128), f32),
                pltpu.VMEM((4 * 32, 256), u32),
                pltpu.VMEM((2, 8, 128), f32),
                pltpu.VMEM((7 * 128, 256), u32),
                pltpu.VMEM((25 * 64, 256), u32),
                pltpu.VMEM((7 * FM // 4, 256), u32),
                pltpu.VMEM((25 * 128, 256), u32),
                pltpu.VMEM((25 * 64, 256), u32),
                pltpu.VMEM((7 * 64, 256), u32),
                pltpu.VMEM((7 * 64, FM // 2), u32),
                pltpu.VMEM((7 * 64, FM // 2), u32),
                pltpu.SMEM((1,), jnp.int32),
                pltpu.SemaphoreType.DMA((2 + len(DMA),)),
            ],
            compiler_params=pltpu.CompilerParams(
                vmem_limit_bytes=100 * 1024 * 1024,
                disable_bounds_checks=not checks,
                disable_semaphore_checks=not checks),
        )(A_x.reshape(S, D), A_wqkv, jnp.transpose(A_w_phi, (1, 2, 0)), A_wo, B_w1, B_w2, B_w3.T, B_w4, gate_w)
        return out.reshape(1, S, D)

    return run


pallas_gated_mix__linear_kernel_hedgehog__mixer_s_mlp__prompt_kernel = build()
```
